```python
import os as _os
_os.environ.setdefault("JAX_PLATFORMS", "cpu")
import jax
import jax.numpy as jnp

def _softmax(x, axis=-1):
    return jax.nn.softmax(x, axis=axis)
def _gelu(x):
    return jax.nn.gelu(x, approximate=True)
def _silu(x):
    return jax.nn.silu(x)
def _sigmoid(x):
    return jax.nn.sigmoid(x)
def _layernorm(x, axis=-1, eps=1e-5):
    m = jnp.mean(x, axis=axis, keepdims=True)
    v = jnp.var(x, axis=axis, keepdims=True)
    return (x - m) / jnp.sqrt(v + eps)
def _scatter_add(tgt, idx, src, axis=0):
    return tgt.at[idx].add(src)
def _segment_sum(src, seg, n):
    return jax.ops.segment_sum(src, seg, n)
class _Rng:
    def __init__(self, key):
        self._k = key
    def _next(self):
        self._k, sub = jax.random.split(self._k)
        return sub
    def normal(self, shape):
        return jax.random.normal(self._next(), shape, dtype=jnp.bfloat16)
    def randint(self, lo, hi, shape):
        return jax.random.randint(self._next(), shape, lo, hi, dtype=jnp.int32)
    def uniform(self, shape, lo=0.0, hi=1.0):
        return jax.random.uniform(self._next(), shape, jnp.bfloat16, lo, hi)
    def permutation(self, n):
        return jax.random.permutation(self._next(), n)


kernel_name = 'recurrent_scan__ssm_conv_s5__geglu_ffn__prompt'

def setup_inputs():
    _rng = _Rng(jax.random.key(int.from_bytes(__import__("os").urandom(4), "little")))
    _w = (lambda a: (lambda t: t.astype(jnp.bfloat16) if jnp.issubdtype(t.dtype, jnp.floating) else t)(jnp.asarray(a)))
    def _A_setup():
        B, S, D = 1, 2048, 640
        P = D
        Lambda_re = -0.5 * jnp.exp((lambda *s: _rng.normal(s) * 0.4)(P))
        Lambda_im = (lambda *s: _rng.normal(s) * 0.4)(P) * 1.0
        B_re = (lambda *s: _rng.normal(s) * 0.4)(P, D) * (D ** -0.5)
        B_im = (lambda *s: _rng.normal(s) * 0.4)(P, D) * (D ** -0.5)
        C_re = (lambda *s: _rng.normal(s) * 0.4)(D, P) * (P ** -0.5)
        C_im = (lambda *s: _rng.normal(s) * 0.4)(D, P) * (P ** -0.5)
        log_dt = (lambda *s: _rng.normal(s) * 0.4)(P) * 0.3 - 2.0
        Dskip = (lambda *s: _rng.normal(s) * 0.4)(D)
        return {
            "x": _w((lambda *s: _rng.normal(s) * 0.05)(B, S, D)),
            "Lambda_re": _w(Lambda_re),
            "Lambda_im": _w(Lambda_im),
            "B_re": _w(B_re),
            "B_im": _w(B_im),
            "C_re": _w(C_re),
            "C_im": _w(C_im),
            "log_dt": _w(log_dt),
            "Dskip": _w(Dskip),
        }
    _A_in = _A_setup()

    def _B_setup():
        B, S, D, F = 1, 2048, 640, 1728
        return {
            "x": _w((lambda *s: _rng.normal(s) * 0.05)(B, S, D)),
            "w_gate": _w((lambda *s: _rng.normal(s) * 0.05)(D, F)),
            "w_up": _w((lambda *s: _rng.normal(s) * 0.05)(D, F)),
            "w_down": _w((lambda *s: _rng.normal(s) * 0.05)(F, D)),
        }
    _B_in = _B_setup()

    return {
        "A_x": _A_in["x"],
        "A_Lambda_re": _A_in["Lambda_re"],
        "A_Lambda_im": _A_in["Lambda_im"],
        "A_B_re": _A_in["B_re"],
        "A_B_im": _A_in["B_im"],
        "A_C_re": _A_in["C_re"],
        "A_C_im": _A_in["C_im"],
        "A_log_dt": _A_in["log_dt"],
        "A_Dskip": _A_in["Dskip"],
        "B_x": _B_in["x"],
        "B_w_gate": _B_in["w_gate"],
        "B_w_up": _B_in["w_up"],
        "B_w_down": _B_in["w_down"],
    }

def reference(A_x, A_Lambda_re, A_Lambda_im, A_B_re, A_B_im, A_C_re, A_C_im, A_log_dt, A_Dskip, B_x, B_w_gate, B_w_up, B_w_down):
    def _A_ref(x, Lambda_re, Lambda_im, B_re, B_im, C_re, C_im, log_dt, Dskip):
        Bsz, L, H = x.shape
        Lam = Lambda_re + 1j * Lambda_im
        Bmat = B_re + 1j * B_im
        Cmat = C_re + 1j * C_im
        dt = jnp.exp(log_dt)
        Lam_bar = jnp.exp(dt * Lam)
        B_bar = ((Lam_bar - 1.0) / Lam)[:, None] * Bmat
        Bu = jnp.einsum("bld,pd->blp", x + 0j, B_bar)
        h = jnp.zeros_like(Bu[:, 0, :])
        hs = []
        for t in range(L):
            h = Lam_bar[None, :] * h + Bu[:, t, :]
            hs.append(h)
        hseq = jnp.stack(hs, 1)
        y = 2.0 * jnp.einsum("blp,dp->bld", hseq, Cmat).real + x * Dskip[None, None, :]
        return y

    def _B_ref(x, w_gate, w_up, w_down):
        return (_gelu(x @ w_gate) * (x @ w_up)) @ w_down

    x = A_x
    xn = _layernorm(x, axis=-1)
    s = _A_ref(xn, A_Lambda_re, A_Lambda_im, A_B_re, A_B_im, A_C_re, A_C_im, A_log_dt, A_Dskip)
    g = _silu(_B_ref(xn, B_w_gate, B_w_up, B_w_down))
    return x + s * g
```

```python
import functools, itertools, math
import jax
import jax.numpy as jnp
from jax import lax
import jax.experimental.pallas as pl
import jax.experimental.pallas.tpu as pltpu

F32 = jnp.float32
BF16 = jnp.bfloat16
T = 128
POINTS4 = (0.35, -0.35, 1.35, -1.35)
POINTS5 = (0.0, 0.618, -0.618, 1.618, -1.618)


def _gelu(x):
    c = math.sqrt(2.0 / math.pi)
    return (0.5 * x) * (1.0 + jnp.tanh(x * (c + (c * 0.044715) * (x * x))))


def _cmul(ar, ai, br, bi):
    return ar * br - ai * bi, ar * bi + ai * br


def _axpy(a, c, b, const=None):
    m = round(abs(c), 9)
    if m == 0:
        return a
    mb = b if m == 1 else b * (m if const is None else const(m))
    return a + mb if c > 0 else a - mb


def _lhs_jobs(out, a1, a2, t, const=None):
    n = len(t)
    g = {}

    def diag(j):
        g[j] = _axpy(a1(j), -t[j], a2(j), const)
        out["d1", j] = g[j].astype(BF16)
        out["d2", j] = a2(j).astype(BF16)

    def pair(j, l):
        q = g[j] + g[l]
        out["q1", j, l] = q.astype(BF16)
        out["q2", j, l] = _axpy(q, t[j] - t[l], a2(j), const).astype(BF16)
        out["q2", l, j] = _axpy(q, t[l] - t[j], a2(l), const).astype(BF16)

    return ([(64, functools.partial(diag, j)) for j in range(n)],
            [(144, functools.partial(pair, j, l)) for j in range(n) for l in range(j + 1, n)])


def _rhs_jobs(out, x1, x2, t, const, raw1=None, raw2=None):
    n = len(t)

    def diag(j):
        out["d1", j] = x1(j).astype(BF16) if raw1 is None else functools.partial(raw1, j)
        if t[j] == 0 and raw2 is not None:
            out["d2", j] = functools.partial(raw2, j)
        else:
            out["d2", j] = _axpy(x2(j), t[j], x1(j), const).astype(BF16)

    def pair(j, l):
        a1, a2, b1, b2 = x1(j), x2(j), x1(l), x2(l)
        d1 = a1 - b1
        w = _axpy(a2 - b2, t[j], d1) * const(1.0 / (t[l] - t[j]))
        out["q1", j, l] = (b1 - w).astype(BF16)
        out["q2", j, l] = w.astype(BF16)
        out["q2", l, j] = (w + d1).astype(BF16)

    return ([(96, functools.partial(diag, j)) for j in range(n)],
            [(176, functools.partial(pair, j, l)) for j in range(n) for l in range(j + 1, n)])


class _Pool:
    def __init__(self, ref, slots, cache):
        self.ref, self.slots, self.where, self.direct, self.seen, self.cache = ref, slots, {}, {}, {}, cache

    def __setitem__(self, key, v):
        if callable(v):
            self.direct[key] = v
        else:
            self.where[key] = next(self.slots)
            self.ref[self.where[key]] = v

    def __getitem__(self, key):
        if key not in self.seen or not self.cache:
            self.seen[key] = self.direct[key]() if key in self.direct else self.ref[self.where[key]]
        return self.seen[key]


class _Values(dict):
    def __getitem__(self, key):
        v = dict.__getitem__(self, key)
        return v() if callable(v) else v


def _merge(*lists):
    keyed = []
    for i, jobs in enumerate(lists):
        total = sum(c for c, _ in jobs)
        acc = 0
        for c, f in jobs:
            keyed.append(((acc + (0.5 * c if i else 0)) / total, i, len(keyed), c, f))
            acc += c
    return [(c, f) for _, _, _, c, f in sorted(keyed, key=lambda k: k[:3])]


def _run(main, *sides):
    for _, f in _merge(main, *sides):
        f()


def make(SEGS=(255, 1), flags=None, LNR=128, SK=8, MIX=False, PLAN=0, CACHE=7):
    def kernel(x_hbm, lre_hbm, lim_hbm, bre_hbm, bim_hbm, cre_hbm, cim_hbm, ldt_hbm, dsk_hbm,
               wg_hbm, wu_hbm, wd_hbm, o_hbm,
               x_v, lre_v, lim_v, ldt_v, dsk_v, bre_v, bim_v, cre_v, cim_v, wg_v, wu_v, wd_v, o_v, s_v, pool_v, act_v, sems, osems):
        S, D = x_hbm.shape
        P = lre_hbm.shape[0]
        F = wg_hbm.shape[0]
        NB, ND, NP, NF = S // T, D // T, P // T, -(-F // T)
        t1, t2 = POINTS4, POINTS5
        started = []

        def fetch(src, dst, r0=None, n=None):
            if r0 is not None:
                src, dst = src.at[pl.ds(r0, n)], dst.at[pl.ds(r0, n)]
            c = pltpu.make_async_copy(src, dst, sems.at[len(started)])
            c.start()
            started.append(c)
            return c

        def wait(*cs):
            for c in cs:
                c.wait()

        c0 = [fetch(x_hbm, x_v, j * T, T) for j in range(4)]
        cx = [None]
        cb = [[fetch(a, b, r0, n) for a, b in ((bre_hbm, bre_v), (bim_hbm, bim_v))] for r0, n in ((4 * T, T), (0, 2 * T), (2 * T, 2 * T))]
        cx += [fetch(x_hbm, x_v, 4 * T * c, 4 * T) for c in range(1, NB // 4)]
        cp = [fetch(a, b) for a, b in ((lre_hbm, lre_v), (lim_hbm, lim_v), (ldt_hbm, ldt_v), (dsk_hbm, dsk_v))]
        late = [cp.pop()]
        cw = [fetch(wg_hbm, wg_v), fetch(wu_hbm, wu_v)]
        c2 = [fetch(cre_hbm, cre_v), fetch(cim_hbm, cim_v), fetch(wd_hbm, wd_v)]

        wait(c0[0])
        x0 = x_v[0:16, 0:T].astype(F32)[0:8]
        never8 = x0 * x0 < 0.0
        never = jnp.concatenate([never8] * (T // 8), 0)
        latest = [None]

        def dot(a, b, rhs_dim):
            latest[0] = lax.dot_general(a, b, (((1,), (rhs_dim,)), ((), ())), preferred_element_type=F32)
            return latest[0]

        dot_nt, dot_nn = functools.partial(dot, rhs_dim=1), functools.partial(dot, rhs_dim=0)
        paced = lambda c: jnp.where(never, latest[0], c)
        plain = lambda c: c
        tile = lambda ref, i, k: ref[i * T:(i + 1) * T, k * T:(k + 1) * T]
        slots = itertools.count()

        xn = {}
        U = [[_Pool(pool_v, slots, CACHE & 1) if c else _Values() for _ in range(3)] for c in range(NB // 4)]

        def lhs1_jobs(c):
            const = paced if c else plain

            def ln(rb):
                if 0 < rb < 4:
                    wait(c0[rb])
                x = x_v[rb * T:(rb + 1) * T, :].astype(F32)
                xc = x - jnp.mean(x, axis=-1, keepdims=True)
                r = lax.rsqrt(jnp.mean(xc * xc, axis=-1, keepdims=True) + const(1e-5))
                for k in range(ND):
                    xn[rb, k] = xc[:, k * T:(k + 1) * T] * r
                for k in (0, 1, 4):
                    U[c][2][rb % 4, k] = xn[rb, k].astype(BF16)

            js = [_lhs_jobs(U[c][k], lambda j, k=k: xn[4 * c + j, k], lambda j, k=k: xn[4 * c + j, 2 + k], t1, const) for k in range(2)]
            return ([(560, functools.partial(ln, rb)) for rb in range(4 * c, 4 * c + 4)]
                    + _merge(js[0][0], js[1][0]) + _merge(js[0][1], js[1][1]))

        def rhs1_jobs(cols, rowsets, pooled):
            Vs, diags, pairs = [], [], []
            for rs in rowsets:
                V = [_Pool(pool_v, slots, CACHE & 2) if pooled else _Values() for _ in range(2)]
                Vs.append((rs, V))
                for k in range(2):
                    d, q = _rhs_jobs(V[k], lambda l, k=k: tile(*cols[l], k).astype(F32), lambda l, k=k: tile(*cols[l], 2 + k).astype(F32),
                                     [t1[j] for j in rs], paced if pooled else plain, lambda l, k=k: tile(*cols[l], k))
                    diags.append(d)
                    pairs.append(q)
            return (cols, Vs), _merge(*diags) + _merge(*pairs)

        def layer1_jobs(c, W, emit):
            cols, Vs = W
            jobs = []
            for rs, V in Vs:
                n = len(rs)
                m = {}
                prod = lambda ku, kv, V=V: dot_nt(U[c][0][ku], V[0][kv]) + dot_nt(U[c][1][ku], V[1][kv])
                rest = lambda j, l: dot_nt(U[c][2][j, 4], tile(*cols[l], 4))

                def diag(a, rs=rs, m=m, prod=prod):
                    m["d1", a] = prod(("d1", rs[a]), ("d1", a))
                    m["d2", a] = prod(("d2", rs[a]), ("d2", a))

                def cell(a, rs=rs, m=m):
                    emit(4 * c + rs[a], a, (m["d1", a] + m["d2", a]) + rest(rs[a], a))

                def pair1(a, b, rs=rs, m=m, prod=prod):
                    m["q"] = prod(("q1", rs[a], rs[b]), ("q1", a, b))
                    m["y"] = ((m["d2", a] - m["d1", b]) + m["q"]) + prod(("q2", rs[a], rs[b]), ("q2", a, b))

                def pair2(a, b, rs=rs, m=m, prod=prod):
                    emit(4 * c + rs[a], b, m["y"] + rest(rs[a], b))
                    emit(4 * c + rs[b], a, ((m["d2", b] - m["d1", a]) + m["q"]) + (rest(rs[b], a) + prod(("q2", rs[b], rs[a]), ("q2", b, a))))

                jobs += [(4, functools.partial(diag, a)) for a in range(n)]
                jobs += [(1, functools.partial(cell, a)) for a in range(n)]
                for a in range(n):
                    for b in range(a + 1, n):
                        jobs += [(4, functools.partial(pair1, a, b)), (4, functools.partial(pair2, a, b))]
            return jobs

        quad, duo = [(0, 1, 2, 3)], [(0, 3), (1, 2)]

        bgroups = (((4,), duo), ((0, 1), quad), ((2, 3), quad))
        WB = [rhs1_jobs([(bre_v, i) for i in tl] + [(bim_v, i) for i in tl], rs, g > 1) for g, (tl, rs) in enumerate(bgroups)]

        def project_jobs(c, g):
            tl = bgroups[g][0]

            def emit(rb, l, v):
                s_v[l // len(tl), tl[l % len(tl)], rb * T:(rb + 1) * T, :] = v
            return layer1_jobs(c, WB[g][0], emit)

        WG = [rhs1_jobs([(wg_v, 4 * g + l) for l in range(4)], quad, True) for g in range(3)]
        WU = [rhs1_jobs([(wu_v, 4 * g + l) for l in range(4)], quad, True) for g in range(3)]

        _run(lhs1_jobs(0))
        wait(*cb[0])
        _run(WB[0][1])
        _run(project_jobs(0, 0))
        wait(*cb[1])
        _run(WB[1][1])
        first = project_jobs(0, 1)
        _run(first[:10])
        wait(*cb[2])
        _run(first[10:], WB[2][1])
        wait(cx[1])
        _run(project_jobs(0, 2), lhs1_jobs(1))
        for c in (1, 2):
            wait(cx[c + 1])
            _run(sum((project_jobs(c, g) for g in range(3)), []), lhs1_jobs(c + 1))
        wait(*cp, *cw)

        row1 = lambda r: r[...].astype(F32).reshape(1, -1)
        lre = row1(lre_v)
        lim = row1(lim_v)
        dt = jnp.exp(row1(ldt_v)).astype(ldt_v.dtype).astype(F32)
        mag = jnp.exp(dt * lre)
        lbr = mag * jnp.cos(dt * lim)
        lbi = mag * jnp.sin(dt * lim)
        den = lre * lre + lim * lim
        cr = 2.0 * ((lbr - 1.0) * lre + lbi * lim) / den
        ci = 2.0 * (lbi * lre - (lbr - 1.0) * lim) / den

        sub = lax.broadcasted_iota(jnp.int32, (8, T), 0)
        zero = jnp.zeros((8, T), F32)
        st = {}

        def scan_jobs(i):
            sl = slice(i * T, (i + 1) * T)
            jobs = []

            def begin():
                st["a"] = (jnp.broadcast_to(lbr[:, sl], (8, T)), jnp.broadcast_to(lbi[:, sl], (8, T)))
                st["c"] = (zero, zero)

            def rows(base, L, k):
                return pl.ds(base + k, 8, stride=L) if L > 1 else pl.ds(base, 8)

            def first(base, L):
                st["h"] = (s_v[0, i, rows(base, L, 0), :], s_v[1, i, rows(base, L, 0), :])

            def steps(base, L, k0, k1, store):
                (ar, ai), (hr, hi) = st["a"], st["h"]
                for k in range(k0, k1):
                    if (k - k0) % 4 == 0:
                        at = (k - k0) * T // SK // 8 * 8
                        ar = jnp.where(never8, latest[0][at:at + 8], st["a"][0])
                    r = rows(base, L, k)
                    hr, hi = (s_v[0, i, r, :] - ai * hi) + ar * hr, (s_v[1, i, r, :] + ai * hr) + ar * hi
                    if store:
                        s_v[0, i, r, :] = hr
                        s_v[1, i, r, :] = hi
                    elif (k - k0) % 4 == 3:
                        s_v[0, i, S:S + 8, :] = hr
                st["h"] = (hr, hi)

            def link(base, L):
                (sr, si), (hr, hi), (c_r, c_i) = st["a"], st["h"], st["c"]
                p, e = None, L
                while e:
                    if e & 1:
                        p = (sr, si) if p is None else _cmul(*p, sr, si)
                    e >>= 1
                    if e:
                        sr, si = _cmul(sr, si, sr, si)
                tr, ti = _cmul(*p, c_r, c_i)
                hr = hr + jnp.where(sub == 0, tr, 0.0)
                hi = hi + jnp.where(sub == 0, ti, 0.0)
                for s in (1, 2, 4):
                    tr, ti = _cmul(*p, pltpu.roll(hr, s, 0), pltpu.roll(hi, s, 0))
                    hr = hr + jnp.where(sub >= s, tr, 0.0)
                    hi = hi + jnp.where(sub >= s, ti, 0.0)
                    if s < 4:
                        p = _cmul(*p, *p)
                er, ei = pltpu.roll(hr, 1, 0), pltpu.roll(hi, 1, 0)
                if L == 1:
                    s_v[0, i, rows(base, L, 0), :] = hr
                    s_v[1, i, rows(base, L, 0), :] = hi
                    st["h"] = (hr, hi)
                else:
                    st["h"] = (jnp.where(sub == 0, c_r, er), jnp.where(sub == 0, c_i, ei))
                st["c"] = (er, ei)

            jobs.append((2, begin))
            base = 0
            for L in SEGS:
                jobs.append((2, functools.partial(first, base, L)))
                jobs += [(8 * SK, functools.partial(steps, base, L, k, min(k + SK, L), False)) for k in range(1, L, SK)]
                jobs.append((100, functools.partial(link, base, L)))
                if L > 1:
                    jobs += [(8 * SK, functools.partial(steps, base, L, k, min(k + SK, L), True)) for k in range(0, L, SK)]
                base += 8 * L
            return jobs

        zr = jnp.max(jnp.where(dt[:, 0:T] < 0.0, 1, 0))
        act = lambda rb, i: act_v[i + zr, rb]

        def tail_jobs():
            lane = lax.broadcasted_iota(jnp.int32, (T, T), 1)
            left = lambda u, j: [u[2][j, 0], u[2][j, 1], u[0]["d2", j], u[1]["d2", j], u[2][j, 4]]
            full = lambda rb, w: functools.reduce(lambda a, b: a + b, [dot_nt(a, w(k)) for k, a in enumerate(left(U[rb // 4], rb % 4))])
            w13 = lambda k: jnp.concatenate([wg_v[13 * T:F, k * T:(k + 1) * T], wu_v[13 * T:F, k * T:(k + 1) * T]], 0)
            keep = {}

            def gate(rb):
                keep[rb] = _gelu(full(rb, lambda k: tile(wg_v, 12, k)))

            def up(rb):
                act_v[12, rb] = keep[rb] * full(rb, lambda k: tile(wu_v, 12, k))

            def both(rb):
                z = full(rb, w13)
                act_v[13, rb] = jnp.where(lane < F - 13 * T, _gelu(z) * pltpu.roll(z, F - 13 * T, 1), 0.0)
            return [(5, functools.partial(f, rb)) for rb in range(NB) for f in (gate, up, both)]

        def glu_jobs(g):
            jobs = []
            for c in range(NB // 4):
                gate = {}

                def emit_g(rb, l, v, gate=gate):
                    gate[rb, l] = _gelu(v)

                def emit_u(rb, l, v, gate=gate):
                    act_v[4 * g + l, rb] = gate[rb, l] * v
                jg, ju = layer1_jobs(c, WG[g][0], emit_g), layer1_jobs(c, WU[g][0], emit_u)
                jobs += [j for pair in zip(jg, ju) for j in pair] if MIX else jg + ju
            return jobs

        half1 = (0, 1, 4, 5, 12, 8, 9)
        half2 = (2, 3, 6, 7, 13, 10, 11)
        VC = [_Pool(pool_v, slots, CACHE & 4) for _ in range(NP)]
        VD = [_Pool(pool_v, slots, CACHE & 4) for _ in half1]

        def vc_jobs():
            jobs = []
            for k in range(NP):
                c12 = {}

                def scale(l, k=k, c12=c12):
                    a, b = tile(cre_v, l, k).astype(F32), tile(cim_v, l, k).astype(F32)
                    u, v = paced(cr[:, k * T:(k + 1) * T]), ci[:, k * T:(k + 1) * T]
                    c12[l] = (a * u - b * v, a * -v - b * u)
                    VC[k]["a2", l] = c12[l][1].astype(BF16)
                d, q = _rhs_jobs(VC[k], lambda l, c12=c12: c12[l][0], lambda l, c12=c12: c12[l][1], t2, paced,
                                 None, lambda l, k=k: VC[k]["a2", l])
                jobs += [j for l in range(ND) for j in ((160, functools.partial(scale, l)), d[l])] + q
            return jobs

        def wd_tile(i, l):
            w = wd_v[i * T:min((i + 1) * T, F), l * T:(l + 1) * T]
            return w if (i + 1) * T <= F else jnp.concatenate([w, jnp.zeros(((i + 1) * T - F, T), BF16)], 0)

        def vd_jobs():
            jobs = []
            for k in range(len(half1)):
                d, q = _rhs_jobs(VD[k], lambda l, k=k: wd_tile(half1[k], l).astype(F32), lambda l, k=k: wd_tile(half2[k], l).astype(F32),
                                 t2, paced, lambda l, k=k: wd_tile(half1[k], l), lambda l, k=k: wd_tile(half2[k], l))
                jobs += d + q
            return jobs

        n2 = len(t2)
        nblk = NB // n2
        UH = [[{} for _ in range(NP)] for _ in range(nblk)]
        UA = [[{} for _ in half1] for _ in range(nblk)]
        hs = lambda z, rb, k: s_v[z, k, rb * T:(rb + 1) * T, :]

        def uh_jobs(b):
            return sum((sum(_lhs_jobs(UH[b][k], lambda j, k=k: hs(0, n2 * b + j, k), lambda j, k=k: hs(1, n2 * b + j, k), t2), []) for k in range(NP)), [])

        def ua_jobs(b):
            return sum((sum(_lhs_jobs(UA[b][k], lambda j, k=k: act(n2 * b + j, half1[k]), lambda j, k=k: act(n2 * b + j, half2[k]), t2), []) for k in range(len(half1))), [])

        flushed = []

        def finish(rb, l, f, y):
            r, sl = slice(rb * T, (rb + 1) * T), slice(l * T, (l + 1) * T)
            hf = 0.5 * f
            o_v[r, sl] = x_v[r, sl].astype(F32) + (y + xn[rb, l] * dsk[:, sl]) * (hf * (1.0 + jnp.tanh(hf)))

        def flush(rb):
            c = pltpu.make_async_copy(o_v.at[pl.ds(rb * T, T)], o_hbm.at[pl.ds(rb * T, T)], osems.at[rb])
            c.start()
            flushed.append(c)

        total = lambda xs: functools.reduce(lambda a, b: a + b, xs)

        def layer2_jobs(Uk, Vk, mm, emit, row_done=None):
            m = {}
            prod = lambda key: total([mm(u[key], v[key]) for u, v in zip(Uk, Vk)])
            nk = len(Uk)

            def d1(j):
                m["d1", j] = prod(("d1", j))

            def d2(j):
                m["d2", j] = prod(("d2", j))
                emit(j, j, m["d1", j] + m["d2", j])

            def q1(j, l):
                m["q"] = prod(("q1", j, l))

            def q2(j, l):
                emit(j, l, ((m["d2", j] - m["d1", l]) + m["q"]) + prod(("q2", j, l)))

            jobs = []
            for j in range(n2):
                jobs += [(nk, functools.partial(d1, j)), (nk, functools.partial(d2, j))]
            for j in range(n2):
                for l in range(j + 1, n2):
                    jobs += [(nk, functools.partial(q1, j, l)), (nk, functools.partial(q2, j, l)), (nk, functools.partial(q2, l, j))]
                if row_done:
                    jobs.append((0, functools.partial(row_done, j)))
            return jobs

        def block_jobs(b):
            ys = {}

            def emit_y(j, l, v):
                ys[j, l] = v
            return (layer2_jobs(UH[b], VC, dot_nt, emit_y),
                    layer2_jobs(UA[b], VD, dot_nn, lambda j, l, v: finish(n2 * b + j, l, v, ys[j, l]), lambda j: flush(n2 * b + j)))

        def rest_jobs(rb):
            ops = {}

            def left():
                ops["h"] = [hs(z, rb, k).astype(BF16) for z in range(2) for k in range(NP)]
                ops["a"] = [act(rb, i).astype(BF16) for i in range(NF)]

            def col(l):
                y = total([dot_nt(a, w) for a, w in zip(ops["h"], [VC[k][key, l] for key in ("d1", "a2") for k in range(NP)])])
                f = total([dot_nn(a, wd_tile(i, l)) for i, a in enumerate(ops["a"])])
                finish(rb, l, f, y)
            return [(0, left)] + [(24, functools.partial(col, l)) for l in range(ND)] + [(0, functools.partial(flush, rb))]

        _run(sum((project_jobs(c, g) for c in (3,) for g in range(3)), []) + tail_jobs(), sum((WG[g][1] + WU[g][1] for g in range(3)), []))
        wait(*c2)
        _run(glu_jobs(0) + glu_jobs(1) + glu_jobs(2), sum((scan_jobs(i) for i in range(NP)), []), vc_jobs() + vd_jobs())
        wait(*late)
        dsk = row1(dsk_v)
        for b in range(nblk):
            yj, fj = block_jobs(b)
            _run(uh_jobs(b))
            _run(ua_jobs(b))
            if PLAN & 1:
                _run([j for pair in zip([j for j in yj], [j for j in fj if j[0]]) for j in pair] + [j for j in fj if not j[0]])
            else:
                _run(yj)
                _run(fj)
        for rb in range(nblk * n2, NB):
            _run(rest_jobs(rb))
        wait(*flushed)

    @jax.jit
    def fn(A_x, A_Lambda_re, A_Lambda_im, A_B_re, A_B_im, A_C_re, A_C_im, A_log_dt, A_Dskip, B_x, B_w_gate, B_w_up, B_w_down):
        _, S, D = A_x.shape
        P = A_Lambda_re.shape[0]
        F = B_w_gate.shape[1]
        hbm = pl.BlockSpec(memory_space=pltpu.HBM)
        args = (A_x.reshape(S, D), A_Lambda_re, A_Lambda_im, A_B_re, A_B_im, A_C_re, A_C_im, A_log_dt, A_Dskip, B_w_gate.T, B_w_up.T, B_w_down)
        out = pl.pallas_call(
            kernel,
            in_specs=[hbm] * 12,
            out_specs=hbm,
            out_shape=jax.ShapeDtypeStruct((S, D), F32),
            scratch_shapes=[pltpu.VMEM((S, D), BF16)] + [pltpu.VMEM((P,), BF16)] * 3 + [pltpu.VMEM((D,), BF16),
                            pltpu.VMEM((P, D), BF16), pltpu.VMEM((P, D), BF16),
                            pltpu.VMEM((D, P), BF16), pltpu.VMEM((D, P), BF16),
                            pltpu.VMEM((F, D), BF16), pltpu.VMEM((F, D), BF16), pltpu.VMEM((F, D), BF16),
                            pltpu.VMEM((S, D), F32), pltpu.VMEM((2, P // T, S + 8, T), F32),
                            pltpu.VMEM((8 * 44 + 45 * 5 + 35 * 7 + 3 * 64, T, T), BF16), pltpu.VMEM((15, S // T, T, T), F32),
                            pltpu.SemaphoreType.DMA((32,)), pltpu.SemaphoreType.DMA((S // T,))],
            compiler_params=pltpu.CompilerParams(vmem_limit_bytes=126 * 2**20, flags=flags),
        )(*args)
        return out.reshape(1, S, D)
    return fn


pallas_recurrent_scan__ssm_conv_s5__geglu_ffn__prompt_kernel = make(CACHE=1)
```

```python
import functools
import itertools
import math

import jax
import jax.experimental.pallas as pl
import jax.experimental.pallas.tpu as pltpu
import jax.numpy as jnp
import numpy as np
from jax import lax

F32 = jnp.float32
BF16 = jnp.bfloat16
T = 128

_RANK40 = (
    ".-...+.... .+.-.-.........+......... +.....+...",
    "+-........ .+.-..................... -+........",
    ".....+-... .....-.........+......... .....+-...",
    ".-....+... .....++.-..-...-......... ......+...",
    "--.-.+.... ...+...........+......... -....-+.+.",
    "--.-.++.+. ...............+......... .....+-.-.",
    "--.-...... ...+..................... +-.-.+-.-.",
    "...+....-. .........-...-..-.++..... ...+......",
    "+.-..-.... ..-.......-.............. +....+.+..",
    "+.-....... ..-...................... -.-..-.-..",
    "+.-..-.+.. ..........-.............. .....-.-..",
    "+....-.... ++.--.....+....-......... +.........",
    "....++.... ....+...............-.... -........+",
    "+...+..... ....+.................... +...+.....",
    ".....+...+ ....................-.... .....-...-",
    ".....+.... +.-+.+.........-....-.... +....+....",
    "....+.+.+- .........-...........-... .-.--....-",
    ".-.-+.+.+- .........-............... .+.++.....",
    "......+.+- .....................-... .+.++.+.++",
    "....-....+ .........+....-.....--.++ .........+",
    ".-....++.. .......+...-............. .--...-...",
    "......++.. .......+................. .++...++..",
    ".--...++.. ...........-............. .++.......",
    "..+....... ..+........-+.-..-....... ..+.......",
    ".+......+. ........-.......+........ ...-..+...",
    "......+.+. ........-......-.....-... ......-.-.",
    ".+.+...... ...-.....-......+........ .+.+......",
    ".+........ .+.-..+-........-........ .+....+...",
    "....-..+.+ ..............-.......+.. ..-.-....-",
    "..-.-..+.+ ..............-.......... ..+.+.....",
    ".......+.+ ......................+.. ..+.+..+.+",
    ".......+.. .......-..-.++........-.. .......+..",
    "..++....-. .............+...+....... ...+...-+.",
    "..++...--. .............+........... .......+-.",
    "..++...... .................+....... ..+-...+-.",
    "........+. ........-........++..+.-. ...+....+.",
    "....+...+. .........-.........+.-.+. ...+.....+",
    "...++..... .........-.........+..... ...-+.....",
    "........++ .....................-.+. ........+-",
    "....+..... ....-....+.........-.--.+ ....+....+",
)
_RANK25 = (
    ".-...+.... .+..+-......... ..+.++",
    "+-........ .+............. .+....",
    ".....+-... ....+-......... ....-.",
    ".-....+... ...+.+--....... ....++",
    "...+....-. .......+-+.+... +-....",
    "+....-.... -.+............ ..+...",
    "....++.... +.............- ..-+..",
    "+...+..... +.............. +.+...",
    ".....+...+ ..............- ...-.-",
    ".....+.... .-+.-+........- ..+..+",
    "....-....+ ............+.- ...+..",
    ".-....++.. ...+..--....... -...--",
    "......++.. ...+........... +..+..",
    ".--...++.. ......--....... +.....",
    "..+....... ........-..+... +--...",
    ".+........ .+..+.......... .++.++",
    ".......+.. ...-..+........ ...+--",
    "..++....-. .......-+..-... +-...+",
    "..++...--. .......-+...... .....-",
    "..++...... ...........-... ..-..-",
    "........+. ..........-..+. +-.+-.",
    "....+...+. .........++..-. +-.+..",
    "...++..... .........++.... .+....",
    "........++ .............-. ....-.",
    "....+..... -........--.++. +..+..",
)
_RANK10 = (
    "+....-.... +.... +.",
    ".....+.... +.... ++",
    ".-....+... .+... .+",
    ".+........ .+... ++",
    "..+....... ..+.. +.",
    ".......+.. ..+.. .+",
    "...+....-. ...+. +.",
    "........+. ...+. ++",
    "....-....+ ....+ .+",
    "....+..... ....+ ++",
)

LATE_AT = 72
NORM_AT = 60
POOL_AT = 80
STAGE_END = 208
POOL_END = 24
HEAD = 3
STAGES = ((3, 4), (5, 6, 7))
LN_ROWS = 16
LEAD = (16, 16)
SEGMENTS = (254, 1, 1)
SCAN_STEPS = 16
BLOCK_ROWS = (144, 128, 128)
STATE_ORDER = [11, 0, 13, 37, 38, 36, 27, 7, 35, 20, 21, 22, 24, 16, 18, 17, 1, 4, 26, 6, 25, 2, 3, 5, 32, 23, 34,
               33, 29, 30, 39, 28, 9, 12, 10, 8, 15, 14, 19, 31]
STATE_ROOM = (20, 24, 20, 25, 10, 24, 25, 20, 15, 24)
GATE_ORDER = [13, 0, 11, 37, 38, 36, 35, 7, 27, 21, 22, 20, 24, 18, 17, 1, 16, 4, 26, 6, 5, 32, 3, 2, 25, 23, 34, 33,
              29, 39, 28, 30, 9, 31, 10, 8, 12, 14, 19, 15]
GATE_ROOM = (25, 15, 25, 0, 0, 25, 0, 0, 10, 0)
UP_ORDER = [11, 0, 13, 37, 24, 36, 35, 7, 20, 27, 21, 38, 16, 17, 6, 4, 22, 1, 26, 18, 25, 2, 3, 5, 32, 23, 34, 33,
            29, 30, 28, 39, 9, 31, 10, 8, 15, 14, 19, 12]
UP_ROOM = (20, 25, 10, 20, 18, 15, 18, 20, 18, 0)
GATE3_ORDER = [5, 19, 9, 18, 23, 22, 2, 1, 20, 12, 24, 21, 10, 16, 3, 8, 17, 11, 15, 0, 4, 14, 13, 7, 6]
GATE3_ROOM = (19, 35, 13, 0, 20, 0)
UP3_ORDER = [5, 22, 19, 9, 18, 23, 2, 1, 20, 12, 24, 21, 10, 16, 15, 3, 8, 17, 11, 0, 7, 14, 4, 13, 6]
UP3_ROOM = (50, 45, 40, 40, 25, 40)
EDGE_ROOM = (50, 60)
DOWN_ORDER = [32, 25, 21, 26, 33, 24, 3, 35, 10, 36, 5, 7, 19, 31, 27, 12, 13, 17, 38, 39, 23, 37, 11, 16, 8, 34, 28,
              18, 0, 20, 9, 2, 22, 4, 15, 30, 14, 29, 6, 1]
DOWN_ROOM = [20, 20, 20, 15, 20, 20, 20, 20, 20, 20, 30, 5, 45, 15, 20, 20, 20, 20, 20, 20, 20, 10, 15, 35, 20, 20,
             20, 5, 20, 20, 20, 20, 20, 20, 15, 30, 15, 20, 20, 20]
READ_ORDER = [26, 21, 33, 32, 3, 25, 10, 35, 5, 7, 19, 36, 31, 39, 13, 38, 24, 27, 11, 12, 37, 23, 17, 16, 8, 28, 18,
              29, 34, 15, 14, 9, 4, 20, 30, 0, 1, 6, 2, 22]
POOL_ORDER = [2, 0, 1, 3]
BUILD_ORDER = [3, 1, 5, 2, 6, 4, 0, 10, 11, 7, 9, 8]


def _gelu2(x):
    c = math.sqrt(2.0 / math.pi)
    return x * (1.0 + jnp.tanh(x * (c + (c * 0.044715) * (x * x))))


def _cmul(ar, ai, br, bi):
    return ar * br - ai * bi, ar * bi + ai * br


def _total(xs):
    return functools.reduce(lambda a, b: a + b, xs)


def _cat(lists):
    return [item for items in lists for item in items]


def _plan(matrix, span=None):
    rows = [{i: int(v) for i, v in enumerate(r) if v} for r in matrix]
    ready = list(range(matrix.shape[1]))
    shared = []
    while True:
        count = {}
        for r in rows:
            for a, b in itertools.combinations(sorted(r), 2):
                if span is None or abs(ready[a] - ready[b]) <= span:
                    count[a, b, r[a] * r[b]] = count.get((a, b, r[a] * r[b]), 0) + 1
        best = max(sorted(count), key=lambda k: (count[k], -abs(ready[k[0]] - ready[k[1]])), default=None)
        if best is None or count[best] < 2:
            break
        a, b, sign = best
        for r in rows:
            if a in r and b in r and r[a] * r[b] == sign:
                r[len(ready)] = r[a]
                del r[a], r[b]
        shared.append(best)
        ready.append(max(ready[a], ready[b]))
    return shared, [sorted(r.items(), key=lambda kv: (ready[kv[0]], kv[0])) for r in rows], ready


class _Sums:
    def __init__(self, plan, source):
        self.shared, self.sums, self.ready = plan
        self.n = len(self.ready) - len(self.shared)
        self.source, self.memo = source, {}

    def var(self, i):
        if i < self.n:
            return self.source(i)
        if i not in self.memo:
            a, b, sign = self.shared[i - self.n]
            self.memo[i] = self.var(a) + self.var(b) if sign > 0 else self.var(a) - self.var(b)
        return self.memo[i]

    def single(self, r):
        (i, sign), *more = self.sums[r]
        return i if not more and sign > 0 and i < self.n else None

    def row(self, r, tap=lambda v: v):
        (i, sign), *more = self.sums[r]
        acc = tap(self.var(i))
        for i, s in more:
            if sign < 0 < s:
                acc, sign = self.var(i) - acc, 1
            else:
                acc = acc + self.var(i) if s == sign else acc - self.var(i)
        return acc if sign > 0 else -acc


class _Scheme:
    def __init__(self, table, order, room, columns=(0, 1, 2)):
        sign = {"+": 1, ".": 0, "-": -1}
        left, right, out = [np.array([[sign[ch] for ch in table[r].split()[k]] for r in order]) for k in columns]
        for m in (left, right):
            flip = m[np.arange(len(m)), (m != 0).argmax(1)] < 0
            m[flip] *= -1
            out[flip] *= -1
        self.rank, self.table_order = len(table), np.argsort(order).tolist()
        self.keys = [tuple(r) for r in left.tolist()]
        self.left, self.right, self.out = _plan(left), _plan(right), _plan(out.T, span=3)
        self.done_at = [max(self.out[2][i] for i, _ in terms) for terms in self.out[1]]
        every = self.rank // len(room)
        self.room = [room[r // every] if r % every == every - 1 else 0 for r in range(self.rank)]


STATE = _Scheme(_RANK40, STATE_ORDER, STATE_ROOM)
GATE = _Scheme(_RANK40, GATE_ORDER, GATE_ROOM)
UP = _Scheme(_RANK40, UP_ORDER, UP_ROOM)
GATE3 = _Scheme(_RANK25, GATE3_ORDER, GATE3_ROOM)
UP3 = _Scheme(_RANK25, UP3_ORDER, UP3_ROOM)
EDGE = _Scheme(_RANK10, range(10), EDGE_ROOM)
DOWN = _Scheme(_RANK40, DOWN_ORDER, DOWN_ROOM, (0, 2, 1))
READ = _Scheme(_RANK40, READ_ORDER, (1,), (0, 2, 1))


class _Values(dict):
    def __setitem__(self, key, v):
        super().__setitem__(key, v if callable(v) else self.keep(v.astype(BF16)))

    def __getitem__(self, key):
        v = super().__getitem__(key)
        return v() if callable(v) else v

    def keep(self, v):
        return v


class _Pool(_Values):
    def __init__(self, ref):
        super().__init__()
        self.ref, self.slots = ref, itertools.count()

    def keep(self, v):
        slot = next(self.slots)
        if self.ref.dtype == BF16:
            self.ref[slot] = v
            return lambda: self.ref[slot]
        at = (slot // 2, pl.ds(slot % 2, T // 2, stride=2), slice(None))
        self.ref[at] = pltpu.bitcast(v, jnp.uint32)
        return lambda: pltpu.bitcast(self.ref[at], BF16)


def _run(main, side=()):
    keyed = []
    for i, jobs in enumerate((main, side)):
        total, acc = sum(c for c, _ in jobs), 0
        for c, job in jobs:
            keyed.append(((acc + 0.5 * c * i) / max(total, 1), i, len(keyed), job))
            acc += c
    for k in sorted(keyed, key=lambda k: k[:3]):
        k[3]()


def _kernel(x_hbm, lre_hbm, lim_hbm, bre_hbm, bim_hbm, cre_hbm, cim_hbm, ldt_hbm, dsk_hbm, wg_hbm, wu_hbm, wd_hbm, o_hbm,
            x_v, bre_v, bim_v, cre_v, cim_v, wg_v, wu_v, wd_v, o_v, s_v, w_pools, c_pools, d_pools, sems,
            lre_v, lim_v, ldt_v, dsk_v):
    S, D = x_hbm.shape
    P, F = lre_hbm.shape[0], wg_hbm.shape[0]
    NS, ND, NP, NF = S // (2 * T), D // T, P // T, -(-F // T)
    KD, extra = NF // 2, F - 13 * T
    rows = lambda i: slice(i * T, (i + 1) * T)
    tile = lambda ref, i, k: ref[rows(i), rows(k)]
    row_vector = lambda ref: ref[...].astype(F32).reshape(1, -1)

    x_tiles = lambda rb, n: (x_hbm, x_v, rb * T, n * T)
    x_stage = lambda pairs: x_tiles(2 * pairs[0], 2 * len(pairs))
    queue = [
        [x_tiles(0, 1)], [x_tiles(1, 1)], [(wg_hbm, wg_v, 13 * T, extra), (wu_hbm, wu_v, 13 * T, extra)],
        [x_tiles(2, 2)], [(wg_hbm, wg_v, 10 * T, 3 * T)], [x_tiles(4, 2)],
        [(bre_hbm, bre_v)], [(bim_hbm, bim_v), x_stage(STAGES[0])], *[[x_stage(pairs)] for pairs in STAGES[1:]],
        [(lre_hbm, lre_v), (lim_hbm, lim_v), (ldt_hbm, ldt_v), (wu_hbm, wu_v, 0, 13 * T), (wg_hbm, wg_v, 0, 10 * T)],
        [(cre_hbm, cre_v), (cim_hbm, cim_v), (wd_hbm, wd_v)], [(dsk_hbm, dsk_v)],
    ]
    flying = []

    def start(sem):
        copies = []
        for src, dst, *at in queue.pop(0):
            if at:
                src, dst = src.at[pl.ds(*at)], dst.at[pl.ds(*at)]
            copies.append(pltpu.make_async_copy(src, dst, sems.at[sem]))
            copies[-1].start()
        flying.append((sem, copies))

    def arrive():
        sem, copies = flying.pop(0)
        for copy in copies:
            copy.wait()
        if queue:
            start(sem)

    for sem in range(sems.shape[0]):
        start(sem)

    arrive()
    x0 = x_v[0:16, 0:T].astype(F32)[0:8]
    never = jnp.concatenate([x0 * x0 < 0.0] * (T // 8), 0)
    latest = [None]

    def dot(a, b, b_dim=1):
        latest[0] = lax.dot_general(a, b, (((1,), (b_dim,)), ((), ())), preferred_element_type=F32)
        return latest[0]

    def paced(v, n=T, at=0):
        return jnp.where(never[:n], latest[0][at:at + n], v)

    def paced_tile(v):
        words = pltpu.bitcast(v, jnp.uint32)
        anchor = lax.bitcast_convert_type(latest[0][:T // 2], jnp.uint32)
        return pltpu.bitcast(jnp.where(never[:T // 2], anchor, words), BF16)

    def operand_jobs(out, plan, keys, source, raw=None, tap=lambda v: v):
        sums = _Sums(plan, source)
        copied = lambda r: None if raw is None else sums.single(r)

        def job(r):
            out[keys[r]] = sums.row(r, tap) if copied(r) is None else functools.partial(raw, copied(r))
        return [(3 + len(sums.sums[r]) if copied(r) is None else 0, functools.partial(job, r)) for r in range(len(keys))]

    def product_jobs(scheme, product, emit):
        m = {}
        sums = _Sums(scheme.out, m.__getitem__)

        def job(r):
            m[r] = product(r)
            for o, at in enumerate(scheme.done_at):
                if at == r:
                    emit(o, sums.row(o))
        return [(scheme.room[r], functools.partial(job, r)) for r in range(scheme.rank)]

    xn, pieces = {}, {}
    U = [_Values() for s in range(NS)]

    def layer_norm(rb, r=0, n=T):
        x = x_v[rb * T + r:rb * T + r + n, :].astype(F32)
        xc = x - jnp.mean(x, axis=-1, keepdims=True)
        eps = paced(1e-5, n) if n < T else 1e-5
        scale = lax.rsqrt(jnp.mean(xc * xc, axis=-1, keepdims=True) + eps)
        for k in range(ND):
            parts = pieces.setdefault((rb, k), [])
            parts.append(xc[:, rows(k)] * scale)
            if r + n == T:
                xn[rb, k] = jnp.concatenate(parts, 0) if len(parts) > 1 else parts[0]

    def norm_jobs(tiles):
        return [(1, functools.partial(layer_norm, rb, r, LN_ROWS)) for rb in tiles for r in range(0, T, LN_ROWS)]

    def left_operands(s):
        _run(operand_jobs(U[s], STATE.left, STATE.keys, lambda i: xn[2 * s + i // ND, i % ND]))

    gate, act = {}, {}
    lane = lax.broadcasted_iota(jnp.int32, (T, T), 1)

    def put_state(z, rb, l, v):
        s_v[z][l][rows(rb), :] = v

    def put_gate(i0, rb, l, v):
        gate[rb, i0 + l] = _gelu2(v)

    def put_act(i0, rb, l, v):
        act[rb, i0 + l] = gate[rb, i0 + l] * v

    def put_edge(rb, _, v):
        act[rb, 13] = jnp.where(lane < extra, _gelu2(v) * pltpu.roll(v, extra, 1), 0.0)

    class Group:
        def __init__(self, scheme, raw, emit, pool=None):
            self.scheme, self.emit, self.tap = scheme, emit, lambda v: v
            self.V = _Values() if pool is None else _Pool(pool)
            tap = (lambda v: v) if pool is None else paced
            self.build = operand_jobs(self.V, scheme.right, range(scheme.rank), lambda i: self.tap(raw(i)).astype(F32), raw, tap)
            if pool is not None:
                self.build = [self.build[r] for r in scheme.table_order]

        def jobs(self, *pairs, emit=None):
            n, emit = len(self.scheme.done_at) // 2, emit or self.emit
            return _cat(product_jobs(self.scheme, lambda r, s=s: dot(U[s][self.scheme.keys[r]], self.V[r]),
                                     lambda o, v, s=s: emit(2 * s + o // n, o % n, v)) for s in pairs)

        def first_jobs(self, pairs, lead):
            _run(self.build[:lead])
            self.tap = paced_tile
            jobs, late = self.jobs(*pairs), [(0, job) for _, job in self.build[lead:]]
            return _cat(jobs[i:i + 4] + late[i:i + 4] for i in range(0, len(jobs), 4))

    def columns(scheme, ref, i0, emit, pool=None):
        n = len(scheme.done_at) // 2
        return Group(scheme, lambda i: tile(ref, i0 + i % n, i // n), emit, pool)

    state = [columns(STATE, ref, 0, functools.partial(put_state, z)) for z, ref in enumerate((bre_v, bim_v))]
    gate3 = columns(GATE3, wg_v, 10, functools.partial(put_gate, 10))
    up3 = columns(UP3, wu_v, 10, functools.partial(put_act, 10))
    edge = Group(EDGE, lambda k: jnp.concatenate([wg_v[13 * T:F, rows(k)], wu_v[13 * T:F, rows(k)]], 0), put_edge)
    glu = [columns(scheme, ref, 5 * g, functools.partial(put, 5 * g), w_pools[2 * g + j])
           for g in range(2) for j, (scheme, ref, put) in enumerate(((GATE, wg_v, put_gate), (UP, wu_v, put_act)))]

    late = []
    hold = lambda group: lambda rb, l, v: late.append((1, lambda: group.emit(rb, l, paced(v))))
    tiles_of = lambda pairs: [2 * s + i for s in pairs for i in range(2)]
    layer_norm(0)
    arrive()
    layer_norm(1)
    left_operands(0)
    arrive()
    _run(edge.build)
    _run(edge.jobs(0, emit=hold(edge)))
    arrive()
    layer_norm(2)
    layer_norm(3)
    left_operands(1)
    _run(edge.jobs(1, emit=hold(edge)))
    arrive()
    _run(gate3.build)
    _run(gate3.jobs(0, emit=hold(gate3)))
    arrive()
    _run(gate3.jobs(1), norm_jobs([4, 5]))
    left_operands(2)
    _run(edge.jobs(2) + gate3.jobs(2, emit=hold(gate3)))
    arrive()
    jobs = state[0].first_jobs(range(HEAD), LEAD[0])
    _run(jobs[:LATE_AT])
    _run(jobs[LATE_AT:], late)
    arrive()
    jobs = state[1].first_jobs(range(HEAD), LEAD[1])
    _run(jobs[:NORM_AT])
    _run(jobs[NORM_AT:], norm_jobs(tiles_of(STAGES[0])))
    arrive()
    for s in STAGES[0]:
        left_operands(s)
    jobs = _cat(group.jobs(s) for s in STAGES[0] for group in (gate3, *state))
    _run(jobs[:STAGE_END], norm_jobs(tiles_of(STAGES[1])))
    arrive()

    lre, lim = row_vector(lre_v), row_vector(lim_v)
    dt = jnp.exp(row_vector(ldt_v)).astype(ldt_v.dtype).astype(F32)
    mag = jnp.exp(dt * lre)
    are, aim = mag * jnp.cos(dt * lim), mag * jnp.sin(dt * lim)
    big = jnp.maximum(jnp.abs(lre), jnp.abs(lim))
    ure, uim = lre / big, lim / big
    den = big * (ure * ure + uim * uim)
    gre = 2.0 * ((are - 1.0) * ure + aim * uim) / den
    gim = 2.0 * (aim * ure - (are - 1.0) * uim) / den

    VC, VD = [_Pool(ref) for ref in c_pools], [_Pool(ref) for ref in d_pools]

    def readout_build(k):
        parts = {}

        def scale(l):
            a, b = tile(cre_v, l, k).astype(F32), tile(cim_v, l, k).astype(F32)
            u, v = paced(gre[:, rows(k)]), gim[:, rows(k)]
            parts[l], parts[ND + l] = a * u - b * v, a * -v - b * u
            for i in (l, ND + l):
                VC[k]["tile", i] = parts[i]
        sums = operand_jobs(VC[k], READ.right, range(READ.rank), parts.__getitem__, lambda i: VC[k]["tile", i], paced)
        return [(13, functools.partial(scale, l)) for l in range(ND)] + [sums[r] for r in READ.table_order]

    def down_tile(i, l):
        w = wd_v[i * T:min((i + 1) * T, F), rows(l)]
        return w if (i + 1) * T <= F else jnp.concatenate([w, jnp.zeros(((i + 1) * T - F, T), BF16)], 0)

    def down_build(k):
        raw = lambda i: down_tile(i // ND * KD + k, i % ND)
        sums = operand_jobs(VD[k], DOWN.right, range(DOWN.rank), lambda i: raw(i).astype(F32), raw, paced)
        return [sums[r] for r in DOWN.table_order]

    _run(up3.build)
    last, before = STAGES[-1], range(STAGES[-1][0])
    for s in last:
        left_operands(s)
    main = jobs[STAGE_END:] + edge.jobs(*before[HEAD:])
    for i, s in enumerate(last):
        main += gate3.jobs(s) + edge.jobs(s) + up3.jobs(s) + state[0].jobs(s) + up3.jobs(*before[i::len(last)]) + state[1].jobs(s)
    _run(main[:POOL_AT])
    _run(main[POOL_AT:len(main) - POOL_END], _cat(glu[i].build for i in POOL_ORDER))
    _run(main[len(main) - POOL_END:])
    arrive()
    builds = [readout_build(k) for k in range(NP)] + [down_build(k) for k in range(KD)]
    _run(_cat(group.jobs(s) for g in range(2) for s in range(NS) for group in glu[2 * g:2 * g + 2]),
         _cat(builds[i] for i in BUILD_ORDER))
    arrive()
    dskip = row_vector(dsk_v)

    sub = lax.broadcasted_iota(jnp.int32, (8, T), 0)
    zero = jnp.zeros((8, T), F32)

    def scan_jobs(i):
        re_v, im_v, st = s_v[0][i], s_v[1][i], {}
        at = lambda base, L, k: pl.ds(base + k, 8, stride=L) if L > 1 else pl.ds(base, 8)

        def begin():
            st["a"] = (jnp.broadcast_to(are[:, rows(i)], (8, T)), jnp.broadcast_to(aim[:, rows(i)], (8, T)))
            st["carry"] = (zero, zero)

        def restart(base, L):
            st["h"] = (re_v[at(base, L, 0), :], im_v[at(base, L, 0), :])

        def steps(base, L, k0, k1, store):
            (ar, ai), (hr, hi) = st["a"], st["h"]
            for k in range(k0, k1):
                if (k - k0) % 4 == 0:
                    ar = paced(st["a"][0], 8, (k - k0) * T // SCAN_STEPS // 8 * 8)
                r = at(base, L, k)
                hr, hi = (re_v[r, :] - ai * hi) + ar * hr, (im_v[r, :] + ai * hr) + ar * hi
                if store:
                    re_v[r, :] = hr
                    im_v[r, :] = hi
                elif (k - k0) % 4 == 3:
                    re_v[S:S + 8, :] = hr
            st["h"] = (hr, hi)

        def link(base, L):
            (sr, si), (hr, hi), (cr, ci) = st["a"], st["h"], st["carry"]
            p, e = None, L
            while e:
                if e & 1:
                    p = (sr, si) if p is None else _cmul(*p, sr, si)
                e >>= 1
                if e:
                    sr, si = _cmul(sr, si, sr, si)
            tr, ti = _cmul(*p, cr, ci)
            hr, hi = hr + jnp.where(sub == 0, tr, 0.0), hi + jnp.where(sub == 0, ti, 0.0)
            for s in (1, 2, 4):
                tr, ti = _cmul(*p, pltpu.roll(hr, s, 0), pltpu.roll(hi, s, 0))
                hr, hi = hr + jnp.where(sub >= s, tr, 0.0), hi + jnp.where(sub >= s, ti, 0.0)
                if s < 4:
                    p = _cmul(*p, *p)
            er, ei = pltpu.roll(hr, 1, 0), pltpu.roll(hi, 1, 0)
            if L == 1:
                re_v[at(base, L, 0), :] = hr
                im_v[at(base, L, 0), :] = hi
            else:
                st["h"] = (jnp.where(sub == 0, cr, er), jnp.where(sub == 0, ci, ei))
            st["carry"] = (er, ei)

        def sweep(base, L, k0, store):
            return [(8 * SCAN_STEPS, functools.partial(steps, base, L, k, min(k + SCAN_STEPS, L), store))
                    for k in range(k0, L, SCAN_STEPS)]

        jobs, base = [(2, begin)], 0
        for L in SEGMENTS:
            jobs += [(2, functools.partial(restart, base, L))] + sweep(base, L, 1, False) + [(100, functools.partial(link, base, L))]
            jobs += sweep(base, L, 0, True) if L > 1 else []
            base += 8 * L
        return jobs

    written = []

    def span(tiles, l, r0, n):
        parts = [tiles[rb, l][max(r0 - rb * T, 0):min(r0 + n - rb * T, T)] for rb in range(r0 // T, -(-(r0 + n) // T))]
        return jnp.concatenate(parts, 0) if len(parts) > 1 else parts[0]

    def finish(r0, n, l, y, f2):
        at = (pl.ds(r0, n), pl.ds(l * T, T))
        h = 0.25 * f2
        o_v[at] = x_v[at].astype(F32) + (y + span(xn, l, r0, n) * dskip[:, rows(l)]) * (h * (1.0 + jnp.tanh(h)))
        written.append(pltpu.make_async_copy(o_v.at[at], o_hbm.at[at], sems.at[0]))
        written[-1].start()

    def layer2_jobs(scheme, source, V, b_dim, emit):
        left = [_Sums(scheme.left, functools.partial(source, k)) for k in range(len(V))]
        return product_jobs(scheme, lambda r: _total([dot(u.row(r).astype(BF16), v[r], b_dim) for u, v in zip(left, V)]), emit)

    def block(r0, n):
        f2 = {}
        ffn = layer2_jobs(DOWN, lambda k, i: span(act, i // 5 * KD + k, r0 + i % 5 * n, n), VD, 0, f2.__setitem__)
        ssm = layer2_jobs(READ, lambda k, i: s_v[i // 5][k][pl.ds(r0 + i % 5 * n, n), :], VC, 1,
                          lambda o, y: finish(r0 + o // ND * n, n, o % ND, y, f2[o]))
        return ffn, ssm

    starts = list(itertools.accumulate(BLOCK_ROWS, lambda r0, n: r0 + 5 * n, initial=0))
    ffn, ssm = zip(*map(block, starts, BLOCK_ROWS))
    _run(_cat(ffn), _cat(scan_jobs(i) for i in range(NP)))
    _run(_cat(ssm))
    r0, n = starts[-1], S - starts[-1]
    states = [s_v[z][k][r0:S, :].astype(BF16) for z in range(2) for k in range(NP)]
    acts = [span(act, i, r0, n).astype(BF16) for i in range(NF)]
    for l in range(ND):
        y = _total([dot(h, VC[i % NP]["tile", i // NP * ND + l]) for i, h in enumerate(states)])
        finish(r0, n, l, y, _total([dot(a, down_tile(i, l), 0) for i, a in enumerate(acts)]))
    for copy in written:
        copy.wait()


@jax.jit
def pallas_recurrent_scan__ssm_conv_s5__geglu_ffn__prompt_kernel(
        A_x, A_Lambda_re, A_Lambda_im, A_B_re, A_B_im, A_C_re, A_C_im, A_log_dt, A_Dskip, B_x, B_w_gate, B_w_up, B_w_down):
    del B_x
    batch, S, D = A_x.shape
    P, F = A_Lambda_re.shape[0], B_w_gate.shape[1]
    assert (batch, S, D, P, F) == (1, 16 * T, 5 * T, 5 * T, 13 * T + T // 2)
    vmem = pltpu.VMEM
    scratch = [
        vmem((S, D), BF16), vmem((P, D), BF16), vmem((P, D), BF16), vmem((D, P), BF16), vmem((D, P), BF16),
        vmem((F, D), BF16), vmem((F, D), BF16), vmem((F, D), BF16), vmem((S, D), F32),
        [[vmem((S + 8, T), F32)] * (P // T)] * 2,
        [vmem((15, T, T), jnp.uint32)] * 4, [vmem((44, T, T), BF16)] * 5, [vmem((34, T, T), BF16)] * 7,
        pltpu.SemaphoreType.DMA((3,)),
        vmem((P,), BF16), vmem((P,), BF16), vmem((P,), BF16), vmem((D,), BF16),
    ]
    hbm = pl.BlockSpec(memory_space=pltpu.HBM)
    out = pl.pallas_call(
        _kernel,
        in_specs=[hbm] * 12,
        out_specs=hbm,
        out_shape=jax.ShapeDtypeStruct((S, D), F32),
        scratch_shapes=scratch,
        compiler_params=pltpu.CompilerParams(vmem_limit_bytes=126 * 2**20),
    )(A_x.reshape(S, D), A_Lambda_re, A_Lambda_im, A_B_re, A_B_im, A_C_re, A_C_im, A_log_dt, A_Dskip,
      B_w_gate.T, B_w_up.T, B_w_down)
    return out.reshape(1, S, D)
```
